```python
import os as _os
_os.environ.setdefault("JAX_PLATFORMS", "cpu")
import jax
import jax.numpy as jnp

def _softmax(x, axis=-1):
    return jax.nn.softmax(x, axis=axis)
def _gelu(x):
    return jax.nn.gelu(x, approximate=True)
def _silu(x):
    return jax.nn.silu(x)
def _sigmoid(x):
    return jax.nn.sigmoid(x)
def _layernorm(x, axis=-1, eps=1e-5):
    m = jnp.mean(x, axis=axis, keepdims=True)
    v = jnp.var(x, axis=axis, keepdims=True)
    return (x - m) / jnp.sqrt(v + eps)
def _scatter_add(tgt, idx, src, axis=0):
    return tgt.at[idx].add(src)
def _segment_sum(src, seg, n):
    return jax.ops.segment_sum(src, seg, n)
class _Rng:
    def __init__(self, key):
        self._k = key
    def _next(self):
        self._k, sub = jax.random.split(self._k)
        return sub
    def normal(self, shape):
        return jax.random.normal(self._next(), shape, dtype=jnp.bfloat16)
    def randint(self, lo, hi, shape):
        return jax.random.randint(self._next(), shape, lo, hi, dtype=jnp.int32)
    def uniform(self, shape, lo=0.0, hi=1.0):
        return jax.random.uniform(self._next(), shape, jnp.bfloat16, lo, hi)
    def permutation(self, n):
        return jax.random.permutation(self._next(), n)


kernel_name = 'concat_heads__mha_block_cached__mha_block_cached__near_ridge'

def setup_inputs():
    _rng = _Rng(jax.random.key(int.from_bytes(__import__("os").urandom(4), "little")))
    _w = (lambda a: (lambda t: t.astype(jnp.bfloat16) if jnp.issubdtype(t.dtype, jnp.floating) else t)(jnp.asarray(a)))
    def _A_setup():
        B, Sq, D = 32, 32, 640
        H, Sk, Dh = 32, 32, 128
        return {
            "x": _w((lambda *s: _rng.normal(s) * 0.8)(B, Sq, D)),
            "k_cache": _w((lambda *s: _rng.normal(s) * 0.8)(B, H, Sk, Dh)),
            "v_cache": _w((lambda *s: _rng.normal(s) * 0.05)(B, H, Sk, Dh)),
            "wq": _w((lambda *s: _rng.normal(s) * 0.8)(D, H * Dh) * (D ** -0.5)),
            "wo": _w((lambda *s: _rng.normal(s) * 0.05)(H * Dh, D) * ((H * Dh) ** -0.5)),
        }
    _A_in = _A_setup()

    def _B_setup():
        B, Sq, D = 32, 32, 640
        H, Sk, Dh = 32, 32, 128
        return {
            "x": _w((lambda *s: _rng.normal(s) * 0.8)(B, Sq, D)),
            "k_cache": _w((lambda *s: _rng.normal(s) * 0.8)(B, H, Sk, Dh)),
            "v_cache": _w((lambda *s: _rng.normal(s) * 0.05)(B, H, Sk, Dh)),
            "wq": _w((lambda *s: _rng.normal(s) * 0.8)(D, H * Dh) * (D ** -0.5)),
            "wo": _w((lambda *s: _rng.normal(s) * 0.05)(H * Dh, D) * ((H * Dh) ** -0.5)),
        }
    _B_in = _B_setup()

    return {
        "A_x": _A_in["x"],
        "A_k_cache": _A_in["k_cache"],
        "A_v_cache": _A_in["v_cache"],
        "A_wq": _A_in["wq"],
        "A_wo": _A_in["wo"],
        "B_x": _B_in["x"],
        "B_k_cache": _B_in["k_cache"],
        "B_v_cache": _B_in["v_cache"],
        "B_wq": _B_in["wq"],
        "B_wo": _B_in["wo"],
    }

def reference(A_x, A_k_cache, A_v_cache, A_wq, A_wo, B_x, B_k_cache, B_v_cache, B_wq, B_wo):
    def _A_ref(x, k_cache, v_cache, wq, wo):
        B, Sq, D = x.shape
        H, Dh = 32, 128
        q = (lambda x, *d: x.transpose(*d))((x @ wq).reshape(B, Sq, H, Dh), 0, 2, 1, 3)
        scores = jnp.einsum("bhqd,bhkd->bhqk", q, k_cache) * (Dh ** -0.5)
        p = _softmax(scores, axis=-1)
        o = jnp.einsum("bhqk,bhkd->bhqd", p, v_cache)
        return (lambda x, *d: x.transpose(*d))(o, 0, 2, 1, 3).reshape(B, Sq, H * Dh) @ wo

    def _B_ref(x, k_cache, v_cache, wq, wo):
        B, Sq, D = x.shape
        H, Dh = 32, 128
        q = (lambda x, *d: x.transpose(*d))((x @ wq).reshape(B, Sq, H, Dh), 0, 2, 1, 3)
        scores = jnp.einsum("bhqd,bhkd->bhqk", q, k_cache) * (Dh ** -0.5)
        p = _softmax(scores, axis=-1)
        o = jnp.einsum("bhqk,bhkd->bhqd", p, v_cache)
        return (lambda x, *d: x.transpose(*d))(o, 0, 2, 1, 3).reshape(B, Sq, H * Dh) @ wo

    a = _A_ref(A_x, A_k_cache, A_v_cache, A_wq, A_wo)
    b = _B_ref(B_x, B_k_cache, B_v_cache, B_wq, B_wo)
    return jnp.concatenate([a, b], axis=-1)
```

```python
import jax
import jax.numpy as jnp
from jax import lax
import jax.experimental.pallas as pl
import jax.experimental.pallas.tpu as pltpu

B, SQ, D, H, SK, DH = 32, 32, 640, 32, 32, 128
M = B * SQ
SCALE = DH ** -0.5
LOG2E = 1.4426950408889634
G = 4
NG = H // G
T = 2 * NG
W = G * DH
LG_NG = NG.bit_length() - 1
QT = 2
PU = 2
MQ = 256
MO = 256
CL = 8
XS = 2
TAILC = 4
NTILE = M // 128

bf16 = jnp.bfloat16
u32 = jnp.uint32
f32 = jnp.float32


def _kernel(xA, kA, vA, wqA, woA, xB, kB, vB, wqB, woB, out,
            xbuf, wqbuf, kbuf, vbuf, wobuf, qall, obuf0, obuf1, acc, ostage,
            sem_x, sem_wq, sem_k, sem_v, sem_wo, sem_out):
    obufs = (obuf0, obuf1)
    xs, ks, vs, wqs, wos = (xA, xB), (kA, kB), (vA, vB), (wqA, wqB), (woA, woB)
    cp = pltpu.make_async_copy
    XR = M // XS

    def br_of(s):
        return s // NG if isinstance(s, int) else lax.shift_right_logical(s, LG_NG)

    def x_copy(br, c):
        return cp(xs[br].at[pl.ds(c * XR, XR)], xbuf.at[br, pl.ds(c * XR, XR)], sem_x.at[br * XS + c])

    def out_copy(br, m0, mc, si):
        return cp(ostage.at[br, pl.ds(m0, mc)], out.at[pl.ds(m0, mc), pl.ds(br * D, D)], sem_out.at[si])

    def wait_wq(s):
        cp(wqA.at[:, pl.ds(0, W)], wqbuf.at[s], sem_wq.at[s]).wait()

    def wait_kv(s):
        cp(kA.at[:, pl.ds(0, G)], kbuf.at[s], sem_k.at[s]).wait()
        cp(vA.at[:, pl.ds(0, G)], vbuf.at[s], sem_v.at[s]).wait()

    def wait_wo(s):
        cp(woA.at[pl.ds(0, W), :], wobuf.at[s], sem_wo.at[s]).wait()

    def _start(b, hg, s, which):
        off = hg * W if isinstance(hg, int) else pl.multiple_of(hg * W, W)
        if which == 'q':
            cp(wqs[b].at[:, pl.ds(off, W)], wqbuf.at[s], sem_wq.at[s]).start()
        else:
            cp(ks[b].at[:, pl.ds(hg * G, G)], kbuf.at[s], sem_k.at[s]).start()
            cp(vs[b].at[:, pl.ds(hg * G, G)], vbuf.at[s], sem_v.at[s]).start()
            cp(wos[b].at[pl.ds(off, W), :], wobuf.at[s], sem_wo.at[s]).start()

    def start(s, which):
        if isinstance(s, int):
            if s < T:
                _start(s // NG, s % NG, s, which)
            return
        br = br_of(s)
        hg = lax.bitwise_and(s, NG - 1)
        for b in (0, 1):
            @pl.when(jnp.logical_and(br == b, s < T))
            def _():
                _start(b, hg, s, which)

    lane_grp = lax.broadcasted_iota(jnp.int32, (SK, 128), 1) // SK
    blk_diag = ((lax.broadcasted_iota(jnp.int32, (64, 128), 0) // (SK // 2))
                == (lax.broadcasted_iota(jnp.int32, (64, 128), 1) // SK))

    def q_pieces(s):
        br = br_of(s)
        pieces = []
        for m0 in range(0, M, MQ):
            def piece(m0=m0):
                qv = jnp.dot(xbuf[br, pl.ds(m0, MQ), :], wqbuf[s], preferred_element_type=f32)
                qall[s, pl.ds(m0 // 2, MQ // 2), :] = pltpu.bitcast(qv.astype(bf16), u32)
            pieces.append(piece)
        return pieces

    def o_pieces(s, par, mo=MO, after=None):
        br = br_of(s)
        pieces = []
        for m0 in range(0, M, mo):
            def piece(m0=m0):
                ov = pltpu.bitcast(obufs[par][pl.ds(m0 // 2, mo // 2), :], bf16)
                r = acc[br, pl.ds(m0, mo), :] + jnp.dot(ov, wobuf[s], preferred_element_type=f32)
                if after is None:
                    acc[br, pl.ds(m0, mo), :] = r
                ostage[br, pl.ds(m0, mo), :] = r.astype(bf16)
                if after is not None:
                    after(m0)
            pieces.append(piece)
        return pieces

    def att_probs(s, hl, j):
        qv = pltpu.bitcast(qall[s, pl.ds(j * 64, 64), pl.ds(hl * DH, DH)], bf16)
        kv = kbuf[s, pl.ds(4 * j, 4), hl].reshape(128, DH)
        st = lax.dot_general(kv, qv, (((1,), (1,)), ((), ())), preferred_element_type=f32)
        mg = jnp.where(lane_grp < 2, jnp.where(lane_grp < 1, st[0:32], st[32:64]),
                       jnp.where(lane_grp < 3, st[64:96], st[96:128]))
        mx = jnp.max(mg, axis=0, keepdims=True)
        p = jnp.exp2((mg - mx) * (SCALE * LOG2E))
        l = jnp.sum(p, axis=0, keepdims=True)
        return (p * (1.0 / l)).astype(bf16)

    def att_out(s, par, hl, j, pb):
        vv = vbuf[s, pl.ds(4 * j, 4), hl].reshape(128, DH)
        pt = jnp.concatenate([pb] * 4, axis=0).T
        pu = jnp.where(blk_diag, pltpu.bitcast(pt, u32), jnp.uint32(0))
        o = jnp.dot(pltpu.bitcast(pu, bf16), vv, preferred_element_type=f32)
        obufs[par][pl.ds(j * 64, 64), pl.ds(hl * DH, DH)] = pltpu.bitcast(o.astype(bf16), u32)

    def step(sq, sa, para, so, paro):
        mm = (q_pieces(sq) if sq is not None else []) + (o_pieces(so, paro) if so is not None else [])
        groups = [(hl, j) for hl in range(G) for j in range(NTILE)]
        nc = len(groups) // CL
        pend = []
        mi = 0
        for c in range(nc):
            ps = [(hl, j, att_probs(sa, hl, j)) for (hl, j) in groups[c * CL:(c + 1) * CL]]
            for hl, j, pb in pend:
                att_out(sa, para, hl, j, pb)
            pend = ps
            while mi < (len(mm) * (c + 1)) // nc:
                mm[mi]()
                mi += 1
        for hl, j, pb in pend:
            att_out(sa, para, hl, j, pb)

    nq_loop = (T - 2) // QT
    s_end = 1 + nq_loop * QT
    np_loop = (T - 1) // PU
    kq = (QT + 1) // 2
    k0 = nq_loop * kq
    assert k0 >= 1 + PU and k0 + PU * np_loop >= T

    start(0, 'q')
    for c in range(XS):
        x_copy(0, c).start()
    acc[...] = jnp.zeros(acc.shape, acc.dtype)

    wait_wq(0)
    x_copy(0, 0).wait()
    for s in range(1, 1 + QT):
        start(s, 'q')
    for c in range(XS):
        x_copy(1, c).start()
    qp = q_pieces(0)
    npc = len(qp) // XS
    for c in range(XS):
        if c > 0:
            x_copy(0, c).wait()
        for p in qp[c * npc:(c + 1) * npc]:
            p()

    def qbody(i, carry):
        s0 = 1 + i * QT
        for d in range(QT):
            wait_wq(s0 + d)

        @pl.when(i == 1)
        def _():
            for c in range(XS):
                x_copy(1, c).wait()
        for d in range(QT):
            start(s0 + QT + d, 'q')
        for d in range(kq):
            start(i * kq + d, 'kv')
        for d in range(QT):
            for p in q_pieces(s0 + d):
                p()
        return carry
    lax.fori_loop(0, nq_loop, qbody, 0)

    rem = list(range(s_end, T))
    for s in range(s_end + QT, T):
        start(s, 'q')
    for s in rem:
        wait_wq(s)
    wait_kv(0)
    for s in rem[:-1]:
        for p in q_pieces(s):
            p()
    step(rem[-1], 0, 0, None, None)

    def pbody(i, carry):
        t = 1 + PU * i
        for d in range(PU):
            wait_kv(t + d)
            wait_wo(t - 1 + d)
        for d in range(PU):
            start(k0 + PU * i + d, 'kv')
        for d in range(PU):
            step(None, t + d, (1 + d) % 2, t - 1 + d, d % 2)

        @pl.when(jnp.logical_and(t - 1 <= NG - 1, NG - 1 < t - 1 + PU))
        def _():
            out_copy(0, 0, M, 0).start()
        return carry
    lax.fori_loop(0, np_loop, pbody, 0)

    prem = list(range(1 + np_loop * PU, T))
    for t in prem:
        wait_kv(t)
        wait_wo(t - 1)
    wait_wo(T - 1)
    for t in prem:
        step(None, t, t % 2, t - 1, (t - 1) % 2)
    mc = M // TAILC
    for p in o_pieces(T - 1, (T - 1) % 2, mo=mc,
                      after=lambda m0: out_copy(1, m0, mc, 1 + m0 // mc).start()):
        p()
    out_copy(0, 0, M, 0).wait()
    for c in range(TAILC):
        out_copy(1, c * mc, mc, 1 + c).wait()


@jax.jit
def pallas_concat_heads__mha_block_cached__mha_block_cached__near_ridge_kernel(
    A_x: jax.Array,
    A_k_cache: jax.Array,
    A_v_cache: jax.Array,
    A_wq: jax.Array,
    A_wo: jax.Array,
    B_x: jax.Array,
    B_k_cache: jax.Array,
    B_v_cache: jax.Array,
    B_wq: jax.Array,
    B_wo: jax.Array,
):
    any_spec = pl.BlockSpec(memory_space=pl.ANY)
    res = pl.pallas_call(
        _kernel,
        out_shape=jax.ShapeDtypeStruct((M, 2 * D), bf16),
        in_specs=[any_spec] * 10,
        out_specs=any_spec,
        scratch_shapes=[
            pltpu.VMEM((2, M, D), bf16),
            pltpu.VMEM((T, D, W), bf16),
            pltpu.VMEM((T, B, G, SK, DH), bf16),
            pltpu.VMEM((T, B, G, SK, DH), bf16),
            pltpu.VMEM((T, W, D), bf16),
            pltpu.VMEM((T, M // 2, W), u32),
            pltpu.VMEM((M // 2, W), u32),
            pltpu.VMEM((M // 2, W), u32),
            pltpu.VMEM((2, M, D), f32),
            pltpu.VMEM((2, M, D), bf16),
            pltpu.SemaphoreType.DMA((2 * XS,)),
            pltpu.SemaphoreType.DMA((T,)),
            pltpu.SemaphoreType.DMA((T,)),
            pltpu.SemaphoreType.DMA((T,)),
            pltpu.SemaphoreType.DMA((T,)),
            pltpu.SemaphoreType.DMA((1 + TAILC,)),
        ],
        compiler_params=pltpu.CompilerParams(
            vmem_limit_bytes=120 * 1024 * 1024, disable_bounds_checks=True),
    )(A_x.reshape(M, D), A_k_cache, A_v_cache, A_wq, A_wo,
      B_x.reshape(M, D), B_k_cache, B_v_cache, B_wq, B_wo)
    return res.reshape(B, SQ, 2 * D)
```

```python
import jax
import jax.numpy as jnp
from jax import lax
import jax.experimental.pallas as pl
import jax.experimental.pallas.tpu as pltpu

B, SQ, D, H, SK, DH = 32, 32, 640, 32, 32, 128
M = B * SQ
SCALE = DH ** -0.5
LOG2E = 1.4426950408889634
G = 4
NG = H // G
T = 2 * NG
W = G * DH
LG_NG = NG.bit_length() - 1
QT = 2
PU = 2
MQ = 256
MO = 256
CL = 8
XC = 256
NXC = M // XC
TAIL = (256, 256, 256, 128, 64, 32, 32)
TOFF = tuple(sum(TAIL[:i]) for i in range(len(TAIL)))
NTILE = M // 128

bf16 = jnp.bfloat16
u32 = jnp.uint32
f32 = jnp.float32


def _kernel(xA, kA, vA, wqA, woA, xB, kB, vB, wqB, woB, out,
            xbuf, wqbuf, kbuf, vbuf, wobuf, qall, obuf0, obuf1, acc, ostage,
            sem_x, sem_wq, sem_k, sem_v, sem_wo, sem_out):
    obufs = (obuf0, obuf1)
    ks, vs, wqs, wos = (kA, kB), (vA, vB), (wqA, wqB), (woA, woB)
    cp = pltpu.make_async_copy

    def br_of(s):
        return s // NG if isinstance(s, int) else lax.shift_right_logical(s, LG_NG)

    def xA_copy(c):
        rows = pl.ds(c * XC, XC) if isinstance(c, int) else pl.ds(pl.multiple_of(c * XC, XC), XC)
        return cp(xA.at[rows], xbuf.at[0, rows], sem_x.at[c])

    def xB_copy():
        return cp(xB, xbuf.at[1], sem_x.at[NXC])

    def out_copy(br, m0, mc, si):
        return cp(ostage.at[br, pl.ds(m0, mc)], out.at[pl.ds(m0, mc), pl.ds(br * D, D)], sem_out.at[si])

    def wait_wq(s):
        cp(wqA.at[:, pl.ds(0, W)], wqbuf.at[s], sem_wq.at[s]).wait()

    def wait_kv(s):
        cp(kA.at[:, pl.ds(0, G)], kbuf.at[s], sem_k.at[s]).wait()
        cp(vA.at[:, pl.ds(0, G)], vbuf.at[s], sem_v.at[s]).wait()

    def wait_wo(s):
        cp(woA.at[pl.ds(0, W), :], wobuf.at[s], sem_wo.at[s]).wait()

    def _start(b, hg, s, which):
        off = hg * W if isinstance(hg, int) else pl.multiple_of(hg * W, W)
        if which == 'q':
            cp(wqs[b].at[:, pl.ds(off, W)], wqbuf.at[s], sem_wq.at[s]).start()
        else:
            cp(ks[b].at[:, pl.ds(hg * G, G)], kbuf.at[s], sem_k.at[s]).start()
            cp(vs[b].at[:, pl.ds(hg * G, G)], vbuf.at[s], sem_v.at[s]).start()
            cp(wos[b].at[pl.ds(off, W), :], wobuf.at[s], sem_wo.at[s]).start()

    def start(s, which):
        if isinstance(s, int):
            if s < T:
                _start(s // NG, s % NG, s, which)
            return
        br = br_of(s)
        hg = lax.bitwise_and(s, NG - 1)
        for b in (0, 1):
            @pl.when(jnp.logical_and(br == b, s < T))
            def _():
                _start(b, hg, s, which)

    lane_grp = lax.broadcasted_iota(jnp.int32, (SK, 128), 1) // SK
    blk_diag = ((lax.broadcasted_iota(jnp.int32, (64, 128), 0) // (SK // 2))
                == (lax.broadcasted_iota(jnp.int32, (64, 128), 1) // SK))

    def q_pieces(s):
        br = br_of(s)
        pieces = []
        for m0 in range(0, M, MQ):
            def piece(m0=m0):
                qv = jnp.dot(xbuf[br, pl.ds(m0, MQ), :], wqbuf[s], preferred_element_type=f32)
                qall[s, pl.ds(m0 // 2, MQ // 2), :] = pltpu.bitcast(qv.astype(bf16), u32)
            pieces.append(piece)
        return pieces

    def o_piece(s, par, br, m0, mc, last=False):
        ov = pltpu.bitcast(obufs[par][pl.ds(m0 // 2, mc // 2), :], bf16)
        r = acc[br, pl.ds(m0, mc), :] + jnp.dot(ov, wobuf[s], preferred_element_type=f32)
        if not last:
            acc[br, pl.ds(m0, mc), :] = r
        ostage[br, pl.ds(m0, mc), :] = r.astype(bf16)

    def o_pieces(s, par, br):
        return [(lambda m0=m0: o_piece(s, par, br, m0, MO)) for m0 in range(0, M, MO)]

    def att_probs(s, hl, j):
        qv = pltpu.bitcast(qall[s, pl.ds(j * 64, 64), pl.ds(hl * DH, DH)], bf16)
        kv = kbuf[s, pl.ds(4 * j, 4), hl].reshape(128, DH)
        st = lax.dot_general(kv, qv, (((1,), (1,)), ((), ())), preferred_element_type=f32)
        mg = jnp.where(lane_grp < 2, jnp.where(lane_grp < 1, st[0:32], st[32:64]),
                       jnp.where(lane_grp < 3, st[64:96], st[96:128]))
        mx = jnp.max(mg, axis=0, keepdims=True)
        p = jnp.exp2((mg - mx) * (SCALE * LOG2E))
        l = jnp.sum(p, axis=0, keepdims=True)
        return (p * (1.0 / l)).astype(bf16)

    def att_out(s, par, hl, j, pb):
        vv = vbuf[s, pl.ds(4 * j, 4), hl].reshape(128, DH)
        pt = jnp.concatenate([pb] * 4, axis=0).T
        pu = jnp.where(blk_diag, pltpu.bitcast(pt, u32), jnp.uint32(0))
        o = jnp.dot(pltpu.bitcast(pu, bf16), vv, preferred_element_type=f32)
        obufs[par][pl.ds(j * 64, 64), pl.ds(hl * DH, DH)] = pltpu.bitcast(o.astype(bf16), u32)

    def step(mm, sa, para, head=False):
        groups = [(hl, j) for hl in range(G) for j in range(NTILE)]
        nc = len(groups) // CL
        pend = []
        mi = 0
        if head:
            mm[0]()
            mi = 1
        for c in range(nc):
            ps = [(hl, j, att_probs(sa, hl, j)) for (hl, j) in groups[c * CL:(c + 1) * CL]]
            for hl, j, pb in pend:
                att_out(sa, para, hl, j, pb)
            pend = ps
            while mi < (len(mm) * (c + 1)) // nc:
                mm[mi]()
                mi += 1
        for hl, j, pb in pend:
            att_out(sa, para, hl, j, pb)

    nq_loop = (T - 2) // QT
    s_end = 1 + nq_loop * QT
    np_loop = (T - 1) // PU
    kq = (QT + 1) // 2
    k0 = nq_loop * kq
    assert k0 >= 1 + PU and k0 + PU * np_loop >= T
    assert PU == 2 and NG % PU == 0 and sum(TAIL) == M

    HW = W // 2

    def wq0_copy(h):
        cols = pl.ds(h * HW, HW)
        return cp(wqA.at[:, cols], wqbuf.at[0, :, cols], sem_wq.at[h * T])

    xA_copy(0).start()
    wq0_copy(0).start()

    def xbody(c, carry):
        @pl.when(c == 0)
        def _():
            wq0_copy(1).start()

        @pl.when(c > 0)
        def _():
            xA_copy(c).start()
        return carry
    lax.fori_loop(0, NXC, xbody, 0)
    for s in range(1, 1 + QT):
        start(s, 'q')
    acc[...] = jnp.zeros(acc.shape, acc.dtype)

    assert MQ == XC and NXC == 4
    xA_copy(0).wait()
    for h in range(2):
        wq0_copy(h).wait()
        cols = pl.ds(h * HW, HW)
        qv = jnp.dot(xbuf[0, pl.ds(0, XC), :], wqbuf[0, :, cols], preferred_element_type=f32)
        qall[0, pl.ds(0, XC // 2), cols] = pltpu.bitcast(qv.astype(bf16), u32)
    qp = q_pieces(0)
    for chunks in ((1,), (2, 3)):
        for c in chunks:
            xA_copy(c).wait()
        for c in chunks:
            qp[c]()
    xB_copy().start()

    def qbody(i, carry):
        s0 = 1 + i * QT
        for d in range(QT):
            wait_wq(s0 + d)

        @pl.when(i == 1)
        def _():
            xB_copy().wait()
        for d in range(QT):
            start(s0 + QT + d, 'q')
        for d in range(kq):
            start(i * kq + d, 'kv')
        for d in range(QT):
            for p in q_pieces(s0 + d):
                p()
        return carry
    lax.fori_loop(0, nq_loop, qbody, 0)

    rem = list(range(s_end, T))
    for s in range(s_end + QT, T):
        start(s, 'q')
    for s in rem:
        wait_wq(s)
    wait_kv(0)
    for s in rem[:-1]:
        for p in q_pieces(s):
            p()
    step(q_pieces(rem[-1]), 0, 0, head=True)

    def pbody(i, carry):
        t = 1 + PU * i
        for d in range(PU):
            wait_kv(t + d)
            wait_wo(t - 1 + d)
        for d in range(PU):
            start(k0 + PU * i + d, 'kv')
        br = br_of(t - 1)
        for d in range(PU):
            step(o_pieces(t - 1 + d, d % 2, br), t + d, (1 + d) % 2, head=(d == 0))

        @pl.when(jnp.logical_and(t - 1 <= NG - 1, NG - 1 < t - 1 + PU))
        def _():
            out_copy(0, 0, M, 0).start()
        return carry
    lax.fori_loop(0, np_loop, pbody, 0)

    prem = list(range(1 + np_loop * PU, T))
    for t in prem:
        wait_kv(t)
        wait_wo(t - 1)
    wait_wo(T - 1)
    for t in prem:
        step(o_pieces(t - 1, (t - 1) % 2, br_of(t - 1)), t, t % 2, head=(t == prem[0]))
    for c, (m0, mc) in enumerate(zip(TOFF, TAIL)):
        o_piece(T - 1, (T - 1) % 2, 1, m0, mc, last=True)
        out_copy(1, m0, mc, 1 + c).start()
    out_copy(0, 0, M, 0).wait()
    for c, (m0, mc) in enumerate(zip(TOFF, TAIL)):
        out_copy(1, m0, mc, 1 + c).wait()


@jax.jit
def pallas_concat_heads__mha_block_cached__mha_block_cached__near_ridge_kernel(
    A_x: jax.Array,
    A_k_cache: jax.Array,
    A_v_cache: jax.Array,
    A_wq: jax.Array,
    A_wo: jax.Array,
    B_x: jax.Array,
    B_k_cache: jax.Array,
    B_v_cache: jax.Array,
    B_wq: jax.Array,
    B_wo: jax.Array,
):
    any_spec = pl.BlockSpec(memory_space=pl.ANY)
    res = pl.pallas_call(
        _kernel,
        out_shape=jax.ShapeDtypeStruct((M, 2 * D), bf16),
        in_specs=[any_spec] * 10,
        out_specs=any_spec,
        scratch_shapes=[
            pltpu.VMEM((2, M, D), bf16),
            pltpu.VMEM((T, D, W), bf16),
            pltpu.VMEM((T, B, G, SK, DH), bf16),
            pltpu.VMEM((T, B, G, SK, DH), bf16),
            pltpu.VMEM((T, W, D), bf16),
            pltpu.VMEM((T, M // 2, W), u32),
            pltpu.VMEM((M // 2, W), u32),
            pltpu.VMEM((M // 2, W), u32),
            pltpu.VMEM((2, M, D), f32),
            pltpu.VMEM((2, M, D), bf16),
            pltpu.SemaphoreType.DMA((NXC + 1,)),
            pltpu.SemaphoreType.DMA((T + 1,)),
            pltpu.SemaphoreType.DMA((T,)),
            pltpu.SemaphoreType.DMA((T,)),
            pltpu.SemaphoreType.DMA((T,)),
            pltpu.SemaphoreType.DMA((1 + len(TAIL),)),
        ],
        compiler_params=pltpu.CompilerParams(
            vmem_limit_bytes=100 * 1024 * 1024, disable_bounds_checks=True),
    )(A_x.reshape(M, D), A_k_cache, A_v_cache, A_wq, A_wo,
      B_x.reshape(M, D), B_k_cache, B_v_cache, B_wq, B_wo)
    return res.reshape(B, SQ, 2 * D)
```
